```python
import os as _os
_os.environ.setdefault("JAX_PLATFORMS", "cpu")
import jax
import jax.numpy as jnp

def _softmax(x, axis=-1):
    return jax.nn.softmax(x, axis=axis)
def _gelu(x):
    return jax.nn.gelu(x, approximate=True)
def _silu(x):
    return jax.nn.silu(x)
def _sigmoid(x):
    return jax.nn.sigmoid(x)
def _layernorm(x, axis=-1, eps=1e-5):
    m = jnp.mean(x, axis=axis, keepdims=True)
    v = jnp.var(x, axis=axis, keepdims=True)
    return (x - m) / jnp.sqrt(v + eps)
def _scatter_add(tgt, idx, src, axis=0):
    return tgt.at[idx].add(src)
def _segment_sum(src, seg, n):
    return jax.ops.segment_sum(src, seg, n)
class _Rng:
    def __init__(self, key):
        self._k = key
    def _next(self):
        self._k, sub = jax.random.split(self._k)
        return sub
    def normal(self, shape):
        return jax.random.normal(self._next(), shape, dtype=jnp.bfloat16)
    def randint(self, lo, hi, shape):
        return jax.random.randint(self._next(), shape, lo, hi, dtype=jnp.int32)
    def uniform(self, shape, lo=0.0, hi=1.0):
        return jax.random.uniform(self._next(), shape, jnp.bfloat16, lo, hi)
    def permutation(self, n):
        return jax.random.permutation(self._next(), n)


kernel_name = 'standalone__linear_kernel_hedgehog__prompt'

def setup_inputs():
    _rng = _Rng(jax.random.key(int.from_bytes(__import__("os").urandom(4), "little")))
    _w = (lambda a: (lambda t: t.astype(jnp.bfloat16) if jnp.issubdtype(t.dtype, jnp.floating) else t)(jnp.asarray(a)))
    B, S, D, H = 1, 2048, 1024, 32
    Dh = D // H
    return {
        "x": _w((lambda *s: _rng.normal(s) * 0.4)(B, S, D)),
        "wqkv": _w((lambda *s: _rng.normal(s) * 0.4)(D, 3 * D)),
        "w_phi": _w((lambda *s: _rng.normal(s) * 0.4)(H, Dh, Dh) * (Dh ** -0.5)),
        "wo": _w((lambda *s: _rng.normal(s) * 0.05)(D, D)),
    }

def reference(x, wqkv, w_phi, wo):
    B, S, D = x.shape
    H = 32; Dh = D // H
    qkv = (lambda x, *d: x.transpose(*d))((x @ wqkv).reshape(B, S, 3, H, Dh), 2, 0, 3, 1, 4)
    q, k, v = qkv[0], qkv[1], qkv[2]
    pq = jnp.einsum("bhsd,hdf->bhsf", q, w_phi)
    pk = jnp.einsum("bhsd,hdf->bhsf", k, w_phi)
    phi_q = jnp.concatenate([_softmax(pq, axis=-1), _softmax(-pq, axis=-1)], axis=-1)
    phi_k = jnp.concatenate([_softmax(pk, axis=-1), _softmax(-pk, axis=-1)], axis=-1)
    kv = jnp.einsum("bhsf,bhsd->bhfd", phi_k, v)
    z  = jnp.einsum("bhsf->bhf", phi_k)
    num = jnp.einsum("bhqf,bhfd->bhqd", phi_q, kv)
    den = jnp.einsum("bhqf,bhf->bhq", phi_q, z)[..., None] + 1e-6
    o = num / den
    return (lambda x, *d: x.transpose(*d))(o, 0, 2, 1, 3).reshape(B, S, D) @ wo
```

```python
import jax
import jax.numpy as jnp
import numpy as np
from jax.experimental import pallas as pl
from jax.experimental.pallas import tpu as pltpu
from functools import partial

NT = (((1,), (1,)), ((), ()))
LOG2E = 1.4426950408889634

def _make(L=512, G=256):
    S, D, H, Dh = 2048, 1024, 32, 32
    NB = S // L
    NG = D // G
    NP = G // 64

    def softmax_pm(p):
        R = p.shape[0]
        p3 = p.reshape(R // 32, 32, p.shape[1])
        mx = jnp.max(p3, axis=1, keepdims=True)
        mn = jnp.min(p3, axis=1, keepdims=True)
        ep = jnp.exp2(p3 - mx)
        em = jnp.exp2(mn - p3)
        sp = jnp.sum(ep, axis=1, keepdims=True)
        sm = jnp.sum(em, axis=1, keepdims=True)
        ep = ep * pl.reciprocal(sp, approx=False)
        em = em * pl.reciprocal(sm, approx=False)
        return ep.reshape(R, -1), em.reshape(R, -1)

    def kernel(x_ref, w_ref, wp_ref, wo_ref, o_ref, wT_ref, kv_ref, z_ref, kvl_ref):
        ph = pl.program_id(0)
        i = pl.program_id(1)

        @pl.when((ph == 0) & (i == 0))
        def _():
            wp = wp_ref[...].astype(jnp.float32)
            rr = jax.lax.broadcasted_iota(jnp.int32, (128, 128), 0) // 32
            cc = jax.lax.broadcasted_iota(jnp.int32, (128, 128), 1) // 32
            msk = rr == cc
            for g in range(8):
                wg = wp[g * 128:(g + 1) * 128, :]
                w4 = jnp.concatenate([wg, wg, wg, wg], axis=1)
                bd = jnp.where(msk, w4, 0.0)
                bdT = bd.T.astype(jnp.bfloat16)
                for t in range(2):
                    c0 = t * D + g * 128
                    r = jax.lax.dot_general(bdT, w_ref[:, c0:c0 + 128], NT, preferred_element_type=jnp.float32)
                    wT_ref[c0:c0 + 128, :] = (r * LOG2E).astype(jnp.bfloat16)
            for g in range(8):
                c0 = 2 * D + g * 128
                wT_ref[c0:c0 + 128, :] = w_ref[:, c0:c0 + 128].T
            kv_ref[...] = jnp.zeros_like(kv_ref)
            z_ref[...] = jnp.zeros_like(z_ref)

        @pl.when(ph == 0)
        def _():
            xb = x_ref[...]
            for g in range(NG):
                pk = jax.lax.dot_general(wT_ref[D + g * G:D + (g + 1) * G, :], xb, NT, preferred_element_type=jnp.float32)
                vT = jax.lax.dot_general(wT_ref[2 * D + g * G:2 * D + (g + 1) * G, :], xb, NT, preferred_element_type=jnp.float32).astype(jnp.bfloat16)
                ep, em = softmax_pm(pk)
                for p in range(NP):
                    pp = g * NP + p
                    phi = jnp.concatenate([ep[p * 64:(p + 1) * 64], em[p * 64:(p + 1) * 64]], axis=0)
                    zs = phi[:, 0:128]
                    for c in range(1, L // 128):
                        zs = zs + phi[:, c * 128:(c + 1) * 128]
                    z_ref[pp] += zs
                    kv_ref[pp] += jax.lax.dot_general(vT[p * 64:(p + 1) * 64], phi.astype(jnp.bfloat16), NT, preferred_element_type=jnp.float32)

        @pl.when((ph == 1) & (i == 0))
        def _():
            r = jax.lax.broadcasted_iota(jnp.int32, (64, 128), 0) // 32
            c = (jax.lax.broadcasted_iota(jnp.int32, (64, 128), 1) % 64) // 32
            m = r == c
            r2 = jax.lax.broadcasted_iota(jnp.int32, (16, 128), 0) // 8
            c2 = (jax.lax.broadcasted_iota(jnp.int32, (16, 128), 1) % 64) // 32
            m2 = r2 == c2
            for pp in range(16):
                kvm = jnp.where(m, kv_ref[pp], 0.0)
                zt = jnp.sum(z_ref[pp].T, axis=0, keepdims=True)
                zb = jnp.where(m2, jnp.broadcast_to(zt, (16, 128)), 0.0)
                kvl_ref[pp] = jnp.concatenate([kvm, zb], axis=0).astype(jnp.bfloat16)

        @pl.when(ph == 1)
        def _():
            xb = x_ref[...]
            os_ = []
            for g in range(NG):
                pq = jax.lax.dot_general(wT_ref[g * G:(g + 1) * G, :], xb, NT, preferred_element_type=jnp.float32)
                ep, em = softmax_pm(pq)
                for p in range(NP):
                    pp = g * NP + p
                    phi = jnp.concatenate([ep[p * 64:(p + 1) * 64], em[p * 64:(p + 1) * 64]], axis=0).astype(jnp.bfloat16)
                    nd = jnp.dot(kvl_ref[pp], phi, preferred_element_type=jnp.float32)
                    rc = pl.reciprocal(nd[64:80] + 1e-6, approx=False)
                    o0 = nd[0:32].reshape(4, 8, L) * rc[0:8][None]
                    o1 = nd[32:64].reshape(4, 8, L) * rc[8:16][None]
                    os_.append(o0.reshape(32, L)); os_.append(o1.reshape(32, L))
            oT = jnp.concatenate(os_, axis=0).astype(jnp.bfloat16)
            o = oT.T
            o_ref[...] = jnp.dot(o, wo_ref[...], preferred_element_type=jnp.float32).astype(jnp.bfloat16)

    def f(x, wqkv, w_phi, wo):
        x2 = x.reshape(S, D)
        wp2 = w_phi.reshape(H * Dh, Dh)
        out = pl.pallas_call(
            kernel,
            grid=(2, NB),
            in_specs=[pl.BlockSpec((L, D), lambda ph, i: (i, 0)),
                      pl.BlockSpec((D, 3 * D), lambda ph, i: (0, 0)),
                      pl.BlockSpec((H * Dh, Dh), lambda ph, i: (0, 0)),
                      pl.BlockSpec((D, D), lambda ph, i: (0, 0))],
            out_specs=pl.BlockSpec((L, D), lambda ph, i: (i * ph, 0)),
            out_shape=jax.ShapeDtypeStruct((S, D), jnp.bfloat16),
            scratch_shapes=[pltpu.VMEM((3 * D, D), jnp.bfloat16),
                            pltpu.VMEM((16, 64, 128), jnp.float32),
                            pltpu.VMEM((16, 128, 128), jnp.float32),
                            pltpu.VMEM((16, 80, 128), jnp.bfloat16)],
            compiler_params=pltpu.CompilerParams(dimension_semantics=("arbitrary", "arbitrary"),
                                                 vmem_limit_bytes=100 * 1024 * 1024),
        )(x2, wqkv, wp2, wo)
        return out.reshape(1, S, D)
    return jax.jit(f)


_IMPL = _make(512, 256)


@jax.jit
def pallas_standalone__linear_kernel_hedgehog__prompt_kernel(
    x: jax.Array,
    wqkv: jax.Array,
    w_phi: jax.Array,
    wo: jax.Array,
):
    return _IMPL(x, wqkv, w_phi, wo)
```

```python
import jax
import jax.numpy as jnp
import numpy as np
from jax.experimental import pallas as pl
from jax.experimental.pallas import tpu as pltpu

NT = (((1,), (1,)), ((), ()))
LOG2E = 1.4426950408889634

def _make(L=512, G=256, OC=1, sched=0):
    S, D, H, Dh = 2048, 1024, 32, 32
    NB = S // L
    NG = D // G
    NP = G // 64
    FG = G // 128

    def softmax_pm(p):
        R = p.shape[0]
        p3 = p.reshape(R // 32, 32, p.shape[1])
        mx = jnp.max(p3, axis=1, keepdims=True)
        mn = jnp.min(p3, axis=1, keepdims=True)
        ep = jnp.exp2(p3 - mx)
        em = jnp.exp2(mn - p3)
        sp = jnp.sum(ep, axis=1, keepdims=True)
        sm = jnp.sum(em, axis=1, keepdims=True)
        ep = ep * pl.reciprocal(sp, approx=False, full_range=False)
        em = em * pl.reciprocal(sm, approx=False, full_range=False)
        return ep.reshape(R, -1), em.reshape(R, -1)

    S_WP = 0
    S_WK = 1
    S_WV = S_WK + NG
    S_WQ = S_WV + NG
    S_X = S_WQ + NG
    S_WO = S_X + NB
    S_OUT = S_WO + 1
    NSEM = S_OUT + NB * OC

    def kernel(x_hbm, w_hbm, wp_hbm, wo_hbm, o_hbm, xv, wraw, wpv, wov, wT, bdT, kv_ref, z_ref, kvl_ref, outv, sems):
        def cp_wp():
            return pltpu.make_async_copy(wp_hbm, wpv, sems.at[S_WP])
        def cp_w(t, g):
            c0 = t * D + g * G
            s = (S_WQ, S_WK, S_WV)[t] + g
            return pltpu.make_async_copy(w_hbm.at[:, pl.ds(c0, G)], wraw.at[:, pl.ds(c0, G)], sems.at[s])
        def cp_x(i):
            return pltpu.make_async_copy(x_hbm.at[pl.ds(i * L, L), :], xv.at[pl.ds(i * L, L), :], sems.at[S_X + i])
        def cp_wo():
            return pltpu.make_async_copy(wo_hbm, wov, sems.at[S_WO])
        def cp_out(i, c):
            r0 = i * L + c * (L // OC)
            return pltpu.make_async_copy(outv.at[pl.ds(r0, L // OC), :], o_hbm.at[pl.ds(r0, L // OC), :], sems.at[S_OUT + i * OC + c])

        def fold(t, g):
            for j in range(FG):
                gg = g * FG + j
                c0 = t * D + gg * 128
                r = jax.lax.dot_general(bdT[gg], wraw[:, c0:c0 + 128], NT, preferred_element_type=jnp.float32)
                wT[c0:c0 + 128, :] = (r * LOG2E).astype(jnp.bfloat16)
        def xpose_v(g):
            for j in range(FG):
                c0 = 2 * D + (g * FG + j) * 128
                wT[c0:c0 + 128, :] = wraw[:, c0:c0 + 128].T

        def phaseA(xb, hook=None):
            for g in range(NG):
                if hook is not None:
                    hook(g)
                    if g == 0:
                        xb = xb()
                pk = jax.lax.dot_general(wT[D + g * G:D + (g + 1) * G, :], xb, NT, preferred_element_type=jnp.float32)
                vT = jax.lax.dot_general(wT[2 * D + g * G:2 * D + (g + 1) * G, :], xb, NT, preferred_element_type=jnp.float32).astype(jnp.bfloat16)
                ep, em = softmax_pm(pk)
                for p in range(NP):
                    pp = g * NP + p
                    phi = jnp.concatenate([ep[p * 64:(p + 1) * 64], em[p * 64:(p + 1) * 64]], axis=0)
                    zs = phi[:, 0:128]
                    for c in range(1, L // 128):
                        zs = zs + phi[:, c * 128:(c + 1) * 128]
                    kvp = jax.lax.dot_general(vT[p * 64:(p + 1) * 64], phi.astype(jnp.bfloat16), NT, preferred_element_type=jnp.float32)
                    if hook is not None:
                        z_ref[pp] = zs
                        kv_ref[pp] = kvp
                    else:
                        z_ref[pp] += zs
                        kv_ref[pp] += kvp

        cp_wp().start()
        cp_w(1, 0).start()
        cp_x(0).start()
        cp_w(2, 0).start()
        if sched == 1:
            for g in range(1, NG):
                cp_w(1, g).start(); cp_w(2, g).start()
            for i in range(1, NB): cp_x(i).start()
            for g in range(NG): cp_w(0, g).start()
            cp_wo().start()
        cp_wp().wait()
        wp = wpv[...].astype(jnp.float32)
        rr = jax.lax.broadcasted_iota(jnp.int32, (128, 128), 0) // 32
        cc = jax.lax.broadcasted_iota(jnp.int32, (128, 128), 1) // 32
        msk = rr == cc
        for g in range(8):
            wg = wp[g * 128:(g + 1) * 128, :]
            w4 = jnp.concatenate([wg, wg, wg, wg], axis=1)
            bdT[g] = jnp.where(msk, w4, 0.0).T.astype(jnp.bfloat16)

        def hook0(g):
            if sched == 0:
                if g + 1 < NG:
                    cp_w(1, g + 1).start(); cp_w(2, g + 1).start()
                else:
                    cp_x(1).start()
                    for gg in range(NG): cp_w(0, gg).start()
            cp_w(1, g).wait()
            fold(1, g)
            cp_w(2, g).wait()
            xpose_v(g)
            if g == 0:
                cp_x(0).wait()
        phaseA(lambda: xv[0:L, :], hook0)

        def bodyA(i, c):
            if sched == 0:
                @pl.when(i + 1 < NB)
                def _():
                    cp_x(i + 1).start()
                @pl.when(i == 1)
                def _():
                    cp_wo().start()
            cp_x(i).wait()
            phaseA(xv[pl.ds(pl.multiple_of(i * L, L), L), :])
            return c
        jax.lax.fori_loop(1, NB, bodyA, 0)

        for g in range(NG):
            cp_w(0, g).wait()
            fold(0, g)
        r = jax.lax.broadcasted_iota(jnp.int32, (64, 128), 0) // 32
        c = (jax.lax.broadcasted_iota(jnp.int32, (64, 128), 1) % 64) // 32
        m = r == c
        r2 = jax.lax.broadcasted_iota(jnp.int32, (16, 128), 0) // 8
        c2 = (jax.lax.broadcasted_iota(jnp.int32, (16, 128), 1) % 64) // 32
        m2 = r2 == c2
        for pp in range(16):
            kvm = jnp.where(m, kv_ref[pp], 0.0)
            zt = jnp.sum(z_ref[pp].T, axis=0, keepdims=True)
            zb = jnp.where(m2, jnp.broadcast_to(zt, (16, 128)), 0.0)
            kvl_ref[pp] = jnp.concatenate([kvm, zb], axis=0).astype(jnp.bfloat16)
        cp_wo().wait()

        def phaseB(i):
            xb = xv[pl.ds(pl.multiple_of(i * L, L), L), :]
            os_ = []
            for g in range(NG):
                pq = jax.lax.dot_general(wT[g * G:(g + 1) * G, :], xb, NT, preferred_element_type=jnp.float32)
                ep, em = softmax_pm(pq)
                for p in range(NP):
                    pp = g * NP + p
                    phi = jnp.concatenate([ep[p * 64:(p + 1) * 64], em[p * 64:(p + 1) * 64]], axis=0).astype(jnp.bfloat16)
                    nd = jnp.dot(kvl_ref[pp], phi, preferred_element_type=jnp.float32)
                    rc = pl.reciprocal(nd[64:80] + 1e-6, approx=False, full_range=False)
                    o0 = nd[0:32].reshape(4, 8, L) * rc[0:8][None]
                    o1 = nd[32:64].reshape(4, 8, L) * rc[8:16][None]
                    os_.append(o0.reshape(32, L)); os_.append(o1.reshape(32, L))
            oT = jnp.concatenate(os_, axis=0).astype(jnp.bfloat16)
            o = oT.T
            LC = L // OC
            for c in range(OC):
                res = jnp.dot(o[c * LC:(c + 1) * LC], wov[...], preferred_element_type=jnp.float32).astype(jnp.bfloat16)
                outv[pl.ds(pl.multiple_of(i * L + c * LC, LC), LC), :] = res
                cp_out(i, c).start()

        def bodyB(i, c):
            phaseB(i)
            return c
        jax.lax.fori_loop(0, NB, bodyB, 0)
        for i in range(NB):
            for c in range(OC):
                cp_out(i, c).wait()

    def f(x, wqkv, w_phi, wo):
        x2 = x.reshape(S, D)
        wp2 = w_phi.reshape(H * Dh, Dh)
        anyspec = pl.BlockSpec(memory_space=pl.ANY)
        out = pl.pallas_call(
            kernel,
            in_specs=[anyspec] * 4,
            out_specs=anyspec,
            out_shape=jax.ShapeDtypeStruct((S, D), jnp.bfloat16),
            scratch_shapes=[pltpu.VMEM((S, D), jnp.bfloat16),
                            pltpu.VMEM((D, 3 * D), jnp.bfloat16),
                            pltpu.VMEM((H * Dh, Dh), jnp.bfloat16),
                            pltpu.VMEM((D, D), jnp.bfloat16),
                            pltpu.VMEM((3 * D, D), jnp.bfloat16),
                            pltpu.VMEM((8, 128, 128), jnp.bfloat16),
                            pltpu.VMEM((16, 64, 128), jnp.float32),
                            pltpu.VMEM((16, 128, 128), jnp.float32),
                            pltpu.VMEM((16, 80, 128), jnp.bfloat16),
                            pltpu.VMEM((S, D), jnp.bfloat16),
                            pltpu.SemaphoreType.DMA((NSEM,))],
            compiler_params=pltpu.CompilerParams(vmem_limit_bytes=100 * 1024 * 1024),
        )(x2, wqkv, wp2, wo)
        return out.reshape(1, S, D)
    return jax.jit(f)


_IMPL = _make(L=512, G=256, OC=4, sched=0)


@jax.jit
def pallas_standalone__linear_kernel_hedgehog__prompt_kernel(
    x: jax.Array,
    wqkv: jax.Array,
    w_phi: jax.Array,
    wo: jax.Array,
):
    return _IMPL(x, wqkv, w_phi, wo)
```

```python
import jax
import jax.numpy as jnp
from jax.experimental import pallas as pl
from jax.experimental.pallas import tpu as pltpu

NT = (((1,), (1,)), ((), ()))
LOG2E = 1.4426950408889634
F32 = jnp.float32
BF = jnp.bfloat16
U32 = jnp.uint32
ORDER = (1, 4, 0, 2, 3, 5, 6)
LEAF_ORDER = [j * 7 + jj for j in ORDER for jj in ORDER]


def pk(v):
    return pltpu.bitcast(v.astype(BF), U32)


def upk(v):
    return pltpu.bitcast(v, BF)


def a_combos(A11, A12, A21, A22):
    return [A11 + A22, A21 + A22, A11, A22, A11 + A12, A21 - A11, A12 - A22]


def b_combos(B11, B12, B21, B22):
    return [B11 + B22, B11, B12 - B22, B21 - B11, B22, B11 + B12, B21 + B22]


def c_assemble(M):
    return (M[0] + M[3] - M[4] + M[6], M[2] + M[4], M[1] + M[3], M[0] - M[1] + M[2] + M[5])


def leaves(Q, comb, emit):
    T = [[comb(Q[b][d], Q[b][2 + d], Q[2 + b][d], Q[2 + b][2 + d]) for d in range(2)] for b in range(2)]
    for j in ORDER:
        l2 = comb(T[0][0][j], T[0][1][j], T[1][0][j], T[1][1][j])
        for jj in ORDER:
            emit(j * 7 + jj, l2[jj])


class Filler:
    def __init__(self, items, nslots, start=0):
        self.gens = []
        for g, n in items:
            self.gens += [g] * n
        self.n = len(self.gens)
        self.nslots = nslots
        self.start = start
        self.done = 0
        self.slot = 0

    def tick(self):
        self.slot += 1
        if self.slot <= self.start:
            return
        want = min(self.n, -(-self.n * (self.slot - self.start) // (self.nslots - self.start)))
        while self.done < want:
            next(self.gens[self.done], None)
            self.done += 1

    def finish(self):
        while self.done < self.n:
            next(self.gens[self.done], None)
            self.done += 1


def strassen2(prod, filler=None):
    sub = [None] * 7
    for j in ORDER:
        M = [None] * 7
        for jj in ORDER:
            M[jj] = prod(j * 7 + jj)
            if filler is not None:
                filler.tick()
        sub[j] = c_assemble(M)
    blk = [[None] * 4 for _ in range(4)]
    for bf in range(4):
        C = c_assemble([sub[j][bf] for j in range(7)])
        b, f = bf // 2, bf % 2
        for ae in range(4):
            a, e = ae // 2, ae % 2
            blk[2 * a + b][2 * e + f] = C[ae]
    return blk


def _make(L=512, FG=4, FGB=8, OC=2, A0G=(2, 2, 4), SJ=3, XS=0, A0S=6, PL=True, TM=0):
    S, D, H, Dh = 2048, 1024, 32, 32
    NB = S // L
    QL = L // 4
    NG = 8 // FG
    NGB = 8 // FGB
    RC = QL // OC
    XB = 49 * (QL // 2)

    def softmax_pm(p):
        R = p.shape[0]
        p3 = p.reshape(R // 32, 32, p.shape[1])
        mx = jnp.max(p3, axis=1, keepdims=True)
        mn = jnp.min(p3, axis=1, keepdims=True)
        ep = jnp.exp2(p3 - mx)
        em = jnp.exp2(mn - p3)
        sp = jnp.sum(ep, axis=1, keepdims=True)
        sm = jnp.sum(em, axis=1, keepdims=True)
        ep = ep * pl.reciprocal(sp, approx=False, full_range=False)
        em = em * pl.reciprocal(sm, approx=False, full_range=False)
        return ep.reshape(R, -1), em.reshape(R, -1)

    S_WP = 0
    S_WK = S_WP + 8
    S_WV = S_WK + 8
    S_WQ = S_WV + 8
    S_X = S_WQ + 1
    S_WO = S_X + NB
    S_OUT = S_WO + 1
    NSEM = S_OUT + NB * OC * 4

    def mo(v, m):
        return v if isinstance(v, int) else pl.multiple_of(v, m)

    def kernel(x_hbm, w_hbm, wp_hbm, wo_hbm, o_hbm, xv, wraw, wpv, wov, wa, wq, wb, xc, bdT, kv_ref, z_ref, kvl, outv, sems):
        def cp_wp():
            return pltpu.make_async_copy(wp_hbm, wpv, sems.at[S_WP])
        def cp_w(t, gi):
            c0 = t * D + sum(A0G[:gi]) * 128
            n = A0G[gi] * 128
            s = (None, S_WK, S_WV)[t] + gi
            return pltpu.make_async_copy(w_hbm.at[:, pl.ds(c0, n)], wraw.at[:, pl.ds(c0, n)], sems.at[s])
        def cp_wqall():
            return pltpu.make_async_copy(w_hbm.at[:, pl.ds(0, D)], wraw.at[:, pl.ds(0, D)], sems.at[S_WQ])
        def cp_x(i):
            return pltpu.make_async_copy(x_hbm.at[pl.ds(i * L, L), :], xv.at[pl.ds(i * L, L), :], sems.at[S_X + i])
        def cp_wo():
            return pltpu.make_async_copy(wo_hbm, wov, sems.at[S_WO])
        def cp_out(i, q, c):
            r0 = i * L + q * QL + c * RC
            return pltpu.make_async_copy(outv.at[pl.ds(r0, RC), :], o_hbm.at[pl.ds(r0, RC), :], sems.at[S_OUT + (i * 4 + q) * OC + c])

        def job_bd(g):
            wg = wpv[g * 128:(g + 1) * 128, :].astype(F32)
            rr = jax.lax.broadcasted_iota(jnp.int32, (128, 128), 0) // 32
            cc = jax.lax.broadcasted_iota(jnp.int32, (128, 128), 1) // 32
            w4 = jnp.concatenate([wg, wg, wg, wg], axis=1)
            t = jnp.where(rr == cc, w4, 0.0).T
            t = jnp.concatenate([t[h * 32 + r:h * 32 + r + 16] for r in (0, 16) for h in range(4)], axis=0)
            bdT[g * 64:(g + 1) * 64, :] = pk(t)
            yield

        def job_fold(t, gg, dst, row0, lstride):
            c0 = mo(t * D + gg * 128, 128)
            b0 = mo(gg * 64, 64)
            wcol = wraw.at[:, pl.ds(c0, 128)]
            bd = bdT.at[pl.ds(b0, 64), :]
            for ri in range(2):
                for cc in (0, 128):
                    lhs = upk(bd[ri * 32:(ri + 1) * 32, :])
                    rhs = jnp.concatenate([wcol[kq * 256 + cc:kq * 256 + cc + 128, :] for kq in range(4)], axis=0)
                    r = jax.lax.dot_general(lhs, rhs, NT, preferred_element_type=F32) * LOG2E
                    Q = [[r[h * 16:(h + 1) * 16, kq * 128:(kq + 1) * 128] for kq in range(4)] for h in range(4)]
                    def emit(l, v, ri=ri, cc=cc):
                        o = row0 + l * lstride + ri * 8
                        dst[o:o + 8, cc:cc + 128] = pk(v)
                    leaves(Q, a_combos, emit)
                    yield

        def job_v(gg):
            wcol = wraw.at[:, pl.ds(mo(2 * D + gg * 128, 128), 128)]
            dst = wa.at[pl.ds(mo(gg * 32, 32), 48 * 256 + 32), :]
            for cc in (0, 128):
                tl = [wcol[kq * 256 + cc:kq * 256 + cc + 128, :].T.astype(F32) for kq in range(4)]
                for ri in range(2):
                    Q = [[tl[kq][h * 32 + ri * 16:h * 32 + ri * 16 + 16] for kq in range(4)] for h in range(4)]
                    def emit(l, v, ri=ri, cc=cc):
                        o = l * 256 + 16 + ri * 8
                        dst[o:o + 8, cc:cc + 128] = pk(v)
                    leaves(Q, a_combos, emit)
                    yield

        def job_o(gg):
            src = wov.at[pl.ds(mo(gg * 128, 128), 128), :]
            dst = wb.at[pl.ds(mo(gg * 16, 16), 48 * 128 + 16), :]
            for ri in range(2):
                for cc in (0, 128):
                    Q = [[src[h * 32 + ri * 16:h * 32 + ri * 16 + 16, nq * 256 + cc:nq * 256 + cc + 128].astype(F32) for nq in range(4)] for h in range(4)]
                    def emit(l, v, ri=ri, cc=cc):
                        o = l * 128 + ri * 8
                        dst[o:o + 8, cc:cc + 128] = pk(v)
                    leaves(Q, b_combos, emit)
                    yield

        def job_q(gg):
            dst = wq.at[pl.ds(mo(gg * 16, 16), 48 * 128 + 16), :]
            return job_fold(0, gg, dst, 0, 128)

        def job_k(gg):
            dst = wa.at[pl.ds(mo(gg * 32, 32), 48 * 256 + 32), :]
            return job_fold(1, gg, dst, 0, 256)

        def run(*jobs):
            for j in jobs:
                for _ in j:
                    pass

        def loop(lo, hi, fn):
            if PL and hi - lo > 1:
                def body(g, c):
                    fn(g)
                    return c
                jax.lax.fori_loop(lo, hi, body, 0)
            else:
                for g in range(lo, hi):
                    fn(g)

        def job_x(xsrc, xdst, off=0):
            for tg in range(QL // 16):
                for cc in (0, 128):
                    Q = [[xsrc[nq * QL + tg * 16:nq * QL + tg * 16 + 16, kq * 256 + cc:kq * 256 + cc + 128].astype(F32) for nq in range(4)] for kq in range(4)]
                    def emit(l, v, tg=tg, cc=cc):
                        o = off + l * (QL // 2) + tg * 8
                        xdst[o:o + 8, cc:cc + 128] = pk(v)
                    leaves(Q, b_combos, emit)
                    yield
        NX = 2 * (QL // 16)

        def phaseA_group(xcur, g0, fg, first, filler=None):
            def prod(l):
                a = upk(wa[l * 256 + g0 * 32:l * 256 + (g0 + fg) * 32, :])
                return jax.lax.dot_general(a, upk(xcur[l * (QL // 2):(l + 1) * (QL // 2), :]), NT, preferred_element_type=F32)
            blk = strassen2(prod, filler)
            for f in range(fg):
                gg = g0 + f
                b = f * 64
                pkk = jnp.concatenate([jnp.concatenate([blk[h][c][b:b + 32] for c in range(4)], axis=1) for h in range(4)], axis=0)
                ep, em = softmax_pm(pkk)
                for p in range(2):
                    pp = gg * 2 + p
                    vT = jnp.concatenate([jnp.concatenate([blk[h][c][b + 32:b + 64] for c in range(4)], axis=1) for h in (2 * p, 2 * p + 1)], axis=0).astype(BF)
                    phi = jnp.concatenate([ep[p * 64:(p + 1) * 64], em[p * 64:(p + 1) * 64]], axis=0)
                    zs = phi[:, 0:128]
                    for c in range(1, L // 128):
                        zs = zs + phi[:, c * 128:(c + 1) * 128]
                    kvp = jax.lax.dot_general(vT, phi.astype(BF), NT, preferred_element_type=F32)
                    if first:
                        z_ref[pp] = zs
                        kv_ref[pp] = kvp
                    else:
                        z_ref[pp] += zs
                        kv_ref[pp] += kvp

        cp_wp().start()
        for gi in range(len(A0G)):
            cp_w(1, gi).start()
            cp_w(2, gi).start()
            if gi == 0:
                cp_x(0).start()
        cp_x(1).start()
        cp_wqall().start()
        cp_wo().start()
        for i in range(2, NB):
            cp_x(i).start()

        cp_wp().wait()
        for g in range(8):
            run(job_bd(g))
        g0 = 0
        for gi, fg in enumerate(A0G):
            cp_w(1, gi).wait()
            if gi == 0:
                loop(g0, g0 + fg, lambda g: run(job_k(g)))
                cp_w(2, gi).wait()
                loop(g0, g0 + fg, lambda g: run(job_v(g)))
                cp_x(0).wait()
                run(job_x(xv.at[0:L, :], xc, 0))
            else:
                for g in range(g0, g0 + fg):
                    run(job_k(g))
                cp_w(2, gi).wait()
                for g in range(g0, g0 + fg):
                    run(job_v(g))
            if gi == len(A0G) - 1:
                cp_x(1).wait()
                fl = Filler([(job_x(xv.at[L:2 * L, :], xc, XB), NX)], 48, start=XS)
            else:
                fl = None
            phaseA_group(xc, g0, fg, True, fl)
            if fl is not None:
                fl.finish()
            g0 += fg

        def bodyA(i, c):
            if SJ > 0:
                @pl.when(i == 1)
                def _():
                    cp_wqall().wait()
                    cp_wo().wait()
            @pl.when(i + 1 < NB)
            def _():
                cp_x(i + 1).wait()
            xw = xc.at[pl.ds(pl.multiple_of(i * XB, XB), 2 * XB), :]
            xcur = xw
            inx = jnp.minimum(i + 1, NB - 1)
            items = [(job_x(xv.at[pl.ds(pl.multiple_of(inx * L, L), L), :], xw, XB), NX)]
            for n in range(SJ):
                gg = jnp.minimum((i - 1) * SJ + n, 7)
                items += [(job_q(gg), 4), (job_o(gg), 4)]
            fl = Filler(items, NG * 49 - 1, start=XS)
            for g in range(NG):
                phaseA_group(xcur, g * FG, FG, False, fl)
            fl.finish()
            return c
        jax.lax.fori_loop(1, NB, bodyA, 0)

        if SJ == 0:
            cp_wqall().wait()
            cp_wo().wait()
        if TM == 0:
            for g in range(SJ * (NB - 1), 8):
                run(job_q(g), job_o(g))
        elif TM == 1:
            for g in range(SJ * (NB - 1), 8):
                run(job_q(g))
            for g in range(SJ * (NB - 1), 8):
                run(job_o(g))
        elif TM == 2:
            for g in range(SJ * (NB - 1), 8):
                run(job_q(g))
            loop(SJ * (NB - 1), 8, lambda g: run(job_o(g)))
        else:
            for g in range(SJ * (NB - 1), 8):
                gq, go = job_q(g), job_o(g)
                for _ in range(4):
                    next(gq); next(go)
        r = jax.lax.broadcasted_iota(jnp.int32, (64, 128), 0) // 32
        c = (jax.lax.broadcasted_iota(jnp.int32, (64, 128), 1) % 64) // 32
        m = r == c
        r2 = jax.lax.broadcasted_iota(jnp.int32, (16, 128), 0) // 8
        c2 = (jax.lax.broadcasted_iota(jnp.int32, (16, 128), 1) % 64) // 32
        m2 = r2 == c2
        ones = jnp.ones((16, 128), BF)
        for pp in range(16):
            kvm = jnp.where(m, kv_ref[pp], 0.0)
            zf = z_ref[pp]
            zh = zf.astype(BF)
            zl = (zf - zh.astype(F32)).astype(BF)
            zt = jax.lax.dot_general(ones, zh, NT, preferred_element_type=F32) + jax.lax.dot_general(ones, zl, NT, preferred_element_type=F32)
            zb = jnp.where(m2, zt, 0.0)
            kvl[pp * 40:(pp + 1) * 40, :] = pk(jnp.concatenate([kvm, zb], axis=0))

        def phaseB(i):
            r0 = pl.multiple_of(i * L, L)
            xcur = xc.at[pl.ds(pl.multiple_of(i * XB, XB), XB), :]
            ow = outv.at[pl.ds(r0, L), :]
            ol = [[] for _ in range(49)]
            for g in range(NGB):
                def prod(l, g=g):
                    a = upk(wq[l * 128 + g * FGB * 16:l * 128 + (g + 1) * FGB * 16, :])
                    return jax.lax.dot_general(a, upk(xcur[l * (QL // 2):(l + 1) * (QL // 2), :]), NT, preferred_element_type=F32)
                blk = strassen2(prod)
                for f in range(FGB):
                    gg = g * FGB + f
                    b = f * 32
                    pq = jnp.concatenate([jnp.concatenate([blk[h][c][b:b + 32] for c in range(4)], axis=1) for h in range(4)], axis=0)
                    ep, em = softmax_pm(pq)
                    nd = []
                    rc = []
                    for p in range(2):
                        pp = gg * 2 + p
                        phi = jnp.concatenate([ep[p * 64:(p + 1) * 64], em[p * 64:(p + 1) * 64]], axis=0).astype(BF)
                        t = jnp.dot(upk(kvl[pp * 40:(pp + 1) * 40, :]), phi, preferred_element_type=F32)
                        rr = pl.reciprocal(t[64:80] + 1e-6, approx=False, full_range=False)
                        nd += [t[0:32], t[32:64]]
                        rc += [rr[0:8], rr[8:16]]
                    for ri in range(2):
                        Q = [[None] * 4 for _ in range(4)]
                        for h in range(4):
                            o = (nd[h][ri * 16:ri * 16 + 16].reshape(2, 8, L) * rc[h][None]).reshape(16, L)
                            for tq in range(4):
                                Q[tq][h] = o[:, tq * QL:(tq + 1) * QL]
                        def emit(l, v):
                            ol[l].append(pk(v))
                        leaves(Q, a_combos, emit)
            OA = [None] * 49
            for l in LEAF_ORDER:
                OA[l] = upk(jnp.concatenate(ol[l], axis=0)).T
            for c in range(OC):
                def prod(l, c=c):
                    return jnp.dot(OA[l][c * RC:(c + 1) * RC], upk(wb[l * 128:(l + 1) * 128, :]), preferred_element_type=F32)
                blk = strassen2(prod)
                for q in range(4):
                    ra = q * QL + c * RC
                    for n in range(4):
                        ow[ra:ra + RC, n * 256:(n + 1) * 256] = blk[q][n].astype(BF)
                    cp_out(i, q, c).start()

        def bodyB(i, c):
            phaseB(i)
            return c
        jax.lax.fori_loop(0, NB, bodyB, 0)
        for i in range(NB):
            for q in range(4):
                for c in range(OC):
                    cp_out(i, q, c).wait()

    def f(x, wqkv, w_phi, wo):
        x2 = x.reshape(S, D)
        wp2 = w_phi.reshape(H * Dh, Dh)
        anyspec = pl.BlockSpec(memory_space=pl.ANY)
        out = pl.pallas_call(
            kernel,
            in_specs=[anyspec] * 4,
            out_specs=anyspec,
            out_shape=jax.ShapeDtypeStruct((S, D), BF),
            scratch_shapes=[pltpu.VMEM((S, D), BF),
                            pltpu.VMEM((D, 3 * D), BF),
                            pltpu.VMEM((H * Dh, Dh), BF),
                            pltpu.VMEM((D, D), BF),
                            pltpu.VMEM((49 * 256, 256), U32),
                            pltpu.VMEM((49 * 128, 256), U32),
                            pltpu.VMEM((49 * 128, 256), U32),
                            pltpu.VMEM(((NB + 1) * XB, 256), U32),
                            pltpu.VMEM((8 * 64, 128), U32),
                            pltpu.VMEM((16, 64, 128), F32),
                            pltpu.VMEM((16, 128, 128), F32),
                            pltpu.VMEM((16 * 40, 128), U32),
                            pltpu.VMEM((S, D), BF),
                            pltpu.SemaphoreType.DMA((NSEM,))],
            compiler_params=pltpu.CompilerParams(vmem_limit_bytes=110 * 1024 * 1024),
        )(x2, wqkv, wp2, wo)
        return out.reshape(1, S, D)
    return jax.jit(f)


_IMPL = _make(FG=8,FGB=8,OC=2,SJ=0,A0G=(3,5),XS=20,TM=2)


@jax.jit
def pallas_standalone__linear_kernel_hedgehog__prompt_kernel(
    x: jax.Array,
    wqkv: jax.Array,
    w_phi: jax.Array,
    wo: jax.Array,
):
    return _IMPL(x, wqkv, w_phi, wo)
```

```python
import jax
import jax.numpy as jnp
import jax.experimental.pallas as pl
import jax.experimental.pallas.tpu as pltpu

S, D, H, DH = 2048, 1024, 32, 32
L = 512
NB = S // L
QL = L // 4
XB = 49 * (QL // 2)
A0G = (3, 5)
SJ = 3
OC = 2
RC = QL // OC

NT = (((1,), (1,)), ((), ()))
LOG2E = 1.4426950408889634
F32 = jnp.float32
BF = jnp.bfloat16
U32 = jnp.uint32
ORDER = (1, 4, 0, 2, 3, 5, 6)
LEAF_ORDER = [j * 7 + jj for j in ORDER for jj in ORDER]

S_WP = 0
S_WK = S_WP + 1
S_WV = S_WK + len(A0G)
S_WQ = S_WV + len(A0G)
S_WO = S_WQ + 1
S_X = S_WO + 1
S_OUT = S_X + NB
NSEM = S_OUT + NB * OC * 4


def _pk(v):
    return pltpu.bitcast(v.astype(BF), U32)


def _upk(v):
    return pltpu.bitcast(v, BF)


def _a_combos(A11, A12, A21, A22):
    return [A11 + A22, A21 + A22, A11, A22, A11 + A12, A21 - A11, A12 - A22]


def _b_combos(B11, B12, B21, B22):
    return [B11 + B22, B11, B12 - B22, B21 - B11, B22, B11 + B12, B21 + B22]


def _c_assemble(M):
    return (M[0] + M[3] - M[4] + M[6], M[2] + M[4], M[1] + M[3],
            M[0] - M[1] + M[2] + M[5])


def _leaves(Q, comb, emit):
    T = [[comb(Q[b][d], Q[b][2 + d], Q[2 + b][d], Q[2 + b][2 + d])
          for d in range(2)] for b in range(2)]
    for j in ORDER:
        l2 = comb(T[0][0][j], T[0][1][j], T[1][0][j], T[1][1][j])
        for jj in ORDER:
            emit(j * 7 + jj, l2[jj])


class _Filler:
    def __init__(self, items, nslots):
        self.steps = []
        for gen, n in items:
            self.steps += [gen] * n
        self.nslots = nslots
        self.done = 0
        self.slot = 0

    def _advance(self, want):
        while self.done < min(want, len(self.steps)):
            next(self.steps[self.done], None)
            self.done += 1

    def tick(self):
        self.slot += 1
        self._advance(-(-len(self.steps) * self.slot // self.nslots))

    def finish(self):
        self._advance(len(self.steps))


def _strassen2(prod, filler=None):
    sub = [None] * 7
    for j in ORDER:
        M = [None] * 7
        for jj in ORDER:
            M[jj] = prod(j * 7 + jj)
            if filler is not None:
                filler.tick()
        sub[j] = _c_assemble(M)
    blk = [[None] * 4 for _ in range(4)]
    for bf in range(4):
        C = _c_assemble([sub[j][bf] for j in range(7)])
        b, f = bf // 2, bf % 2
        for ae in range(4):
            a, e = ae // 2, ae % 2
            blk[2 * a + b][2 * e + f] = C[ae]
    return blk


def _softmax_pm(p):
    R = p.shape[0]
    p3 = p.reshape(R // 32, 32, p.shape[1])
    mx = jnp.max(p3, axis=1, keepdims=True)
    mn = jnp.min(p3, axis=1, keepdims=True)
    ep = jnp.exp2(p3 - mx)
    em = jnp.exp2(mn - p3)
    sp = jnp.sum(ep, axis=1, keepdims=True)
    sm = jnp.sum(em, axis=1, keepdims=True)
    ep = ep * pl.reciprocal(sp, approx=False, full_range=False)
    em = em * pl.reciprocal(sm, approx=False, full_range=False)
    return ep.reshape(R, -1), em.reshape(R, -1)


def _mo(v, m):
    return v if isinstance(v, int) else pl.multiple_of(v, m)


def _run(*jobs):
    for job in jobs:
        for _ in job:
            pass


def _loop(lo, hi, fn):
    def body(g, c):
        fn(g)
        return c
    jax.lax.fori_loop(lo, hi, body, 0)


def _kernel(x_hbm, w_hbm, wp_hbm, wo_hbm, o_hbm,
            xv, wraw, wpv, wov, wa, wq, wb, xc, bdT, kv_ref, z_ref, kvl, outv, sems):
    def cp_wp():
        return pltpu.make_async_copy(wp_hbm, wpv, sems.at[S_WP])

    def cp_w(t, gi):
        c0 = t * D + sum(A0G[:gi]) * 128
        n = A0G[gi] * 128
        s = (S_WK if t == 1 else S_WV) + gi
        return pltpu.make_async_copy(w_hbm.at[:, pl.ds(c0, n)], wraw.at[:, pl.ds(c0, n)], sems.at[s])

    def cp_wq():
        return pltpu.make_async_copy(w_hbm.at[:, pl.ds(0, D)], wraw.at[:, pl.ds(0, D)], sems.at[S_WQ])

    def cp_x(i):
        return pltpu.make_async_copy(x_hbm.at[pl.ds(i * L, L), :], xv.at[pl.ds(i * L, L), :],
                                     sems.at[S_X + i])

    def cp_wo():
        return pltpu.make_async_copy(wo_hbm, wov, sems.at[S_WO])

    def cp_out(i, q, c):
        r0 = i * L + q * QL + c * RC
        return pltpu.make_async_copy(outv.at[pl.ds(r0, RC), :], o_hbm.at[pl.ds(r0, RC), :],
                                     sems.at[S_OUT + (i * 4 + q) * OC + c])

    def job_bd(g):
        wg = wpv[g * 128:(g + 1) * 128, :].astype(F32)
        rr = jax.lax.broadcasted_iota(jnp.int32, (128, 128), 0) // 32
        cc = jax.lax.broadcasted_iota(jnp.int32, (128, 128), 1) // 32
        w4 = jnp.concatenate([wg, wg, wg, wg], axis=1)
        t = jnp.where(rr == cc, w4, 0.0).T
        t = jnp.concatenate([t[h * 32 + r:h * 32 + r + 16] for r in (0, 16) for h in range(4)], axis=0)
        bdT[g * 64:(g + 1) * 64, :] = _pk(t)
        yield

    def job_fold(t, gg, dst, lstride):
        wcol = wraw.at[:, pl.ds(_mo(t * D + gg * 128, 128), 128)]
        bd = bdT.at[pl.ds(_mo(gg * 64, 64), 64), :]
        for ri in range(2):
            for cc in (0, 128):
                lhs = _upk(bd[ri * 32:(ri + 1) * 32, :])
                rhs = jnp.concatenate([wcol[kq * 256 + cc:kq * 256 + cc + 128, :] for kq in range(4)], axis=0)
                r = jax.lax.dot_general(lhs, rhs, NT, preferred_element_type=F32) * LOG2E
                Q = [[r[h * 16:(h + 1) * 16, kq * 128:(kq + 1) * 128] for kq in range(4)] for h in range(4)]

                def emit(l, v, ri=ri, cc=cc):
                    o = l * lstride + ri * 8
                    dst[o:o + 8, cc:cc + 128] = _pk(v)
                _leaves(Q, _a_combos, emit)
                yield

    def job_k(gg):
        return job_fold(1, gg, wa.at[pl.ds(_mo(gg * 32, 32), 48 * 256 + 32), :], 256)

    def job_q(gg):
        return job_fold(0, gg, wq.at[pl.ds(_mo(gg * 16, 16), 48 * 128 + 16), :], 128)

    def job_v(gg):
        wcol = wraw.at[:, pl.ds(_mo(2 * D + gg * 128, 128), 128)]
        dst = wa.at[pl.ds(_mo(gg * 32, 32), 48 * 256 + 32), :]
        for cc in (0, 128):
            tl = [wcol[kq * 256 + cc:kq * 256 + cc + 128, :].T.astype(F32) for kq in range(4)]
            for ri in range(2):
                Q = [[tl[kq][h * 32 + ri * 16:h * 32 + ri * 16 + 16] for kq in range(4)] for h in range(4)]

                def emit(l, v, ri=ri, cc=cc):
                    o = l * 256 + 16 + ri * 8
                    dst[o:o + 8, cc:cc + 128] = _pk(v)
                _leaves(Q, _a_combos, emit)
                yield

    def job_o(gg):
        src = wov.at[pl.ds(_mo(gg * 128, 128), 128), :]
        dst = wb.at[pl.ds(_mo(gg * 16, 16), 48 * 128 + 16), :]
        for ri in range(2):
            for cc in (0, 128):
                Q = [[src[h * 32 + ri * 16:h * 32 + ri * 16 + 16, nq * 256 + cc:nq * 256 + cc + 128].astype(F32)
                      for nq in range(4)] for h in range(4)]

                def emit(l, v, ri=ri, cc=cc):
                    o = l * 128 + ri * 8
                    dst[o:o + 8, cc:cc + 128] = _pk(v)
                _leaves(Q, _b_combos, emit)
                yield

    def job_x(xsrc, xdst, row0):
        for tg in range(QL // 16):
            for cc in (0, 128):
                Q = [[xsrc[nq * QL + tg * 16:nq * QL + tg * 16 + 16, kq * 256 + cc:kq * 256 + cc + 128].astype(F32)
                      for nq in range(4)] for kq in range(4)]

                def emit(l, v, tg=tg, cc=cc):
                    o = row0 + l * (QL // 2) + tg * 8
                    xdst[o:o + 8, cc:cc + 128] = _pk(v)
                _leaves(Q, _b_combos, emit)
                yield
    NX = 2 * (QL // 16)

    def phase_a(xcur, g0, fg, first, filler=None):
        def prod(l):
            a = _upk(wa[l * 256 + g0 * 32:l * 256 + (g0 + fg) * 32, :])
            b = _upk(xcur[l * (QL // 2):(l + 1) * (QL // 2), :])
            return jax.lax.dot_general(a, b, NT, preferred_element_type=F32)
        blk = _strassen2(prod, filler)
        for f in range(fg):
            gg = g0 + f
            b = f * 64
            pk = jnp.concatenate([jnp.concatenate([blk[h][c][b:b + 32] for c in range(4)], axis=1)
                                  for h in range(4)], axis=0)
            ep, em = _softmax_pm(pk)
            for p in range(2):
                pp = gg * 2 + p
                vT = jnp.concatenate([jnp.concatenate([blk[h][c][b + 32:b + 64] for c in range(4)], axis=1)
                                      for h in (2 * p, 2 * p + 1)], axis=0).astype(BF)
                phi = jnp.concatenate([ep[p * 64:(p + 1) * 64], em[p * 64:(p + 1) * 64]], axis=0)
                zs = phi[:, 0:128]
                for c in range(1, L // 128):
                    zs = zs + phi[:, c * 128:(c + 1) * 128]
                kvp = jax.lax.dot_general(vT, phi.astype(BF), NT, preferred_element_type=F32)
                if first:
                    z_ref[pp] = zs
                    kv_ref[pp] = kvp
                else:
                    z_ref[pp] += zs
                    kv_ref[pp] += kvp

    cp_wp().start()
    for gi in range(len(A0G)):
        cp_w(1, gi).start()
        cp_w(2, gi).start()
        if gi == 0:
            cp_x(0).start()
    cp_x(1).start()
    cp_wq().start()
    cp_wo().start()
    for i in range(2, NB):
        cp_x(i).start()

    cp_wp().wait()
    for g in range(8):
        _run(job_bd(g))
    g0 = 0
    for gi, fg in enumerate(A0G):
        cp_w(1, gi).wait()
        if gi == 0:
            _loop(g0, g0 + fg, lambda g: _run(job_k(g)))
            cp_w(2, gi).wait()
            _loop(g0, g0 + fg, lambda g: _run(job_v(g)))
            cp_x(0).wait()
            _run(job_x(xv.at[0:L, :], xc, 0))
        else:
            for g in range(g0, g0 + fg):
                _run(job_k(g))
            cp_w(2, gi).wait()
            for g in range(g0, g0 + fg):
                _run(job_v(g))
        fl = None
        if gi == len(A0G) - 1:
            cp_x(1).wait()
            fl = _Filler([(job_x(xv.at[L:2 * L, :], xc, XB), NX)], 48)
        phase_a(xc, g0, fg, True, fl)
        if fl is not None:
            fl.finish()
        g0 += fg

    def body_a(i, c):
        @pl.when(i == 1)
        def _():
            cp_wq().wait()
            cp_wo().wait()

        @pl.when(i + 1 < NB)
        def _():
            cp_x(i + 1).wait()
        xw = xc.at[pl.ds(pl.multiple_of(i * XB, XB), 2 * XB), :]
        inx = jnp.minimum(i + 1, NB - 1)
        items = [(job_x(xv.at[pl.ds(pl.multiple_of(inx * L, L), L), :], xw, XB), NX)]
        for n in range(SJ):
            items.append((job_q(jnp.minimum((i - 1) * SJ + n, 7)), 4))
        fl = _Filler(items, 48)
        phase_a(xw, 0, 8, False, fl)
        fl.finish()
        return c
    jax.lax.fori_loop(1, NB, body_a, 0)

    for g in range(SJ * (NB - 1), 8):
        _run(job_q(g))
    _loop(0, 8, lambda g: _run(job_o(g)))
    r = jax.lax.broadcasted_iota(jnp.int32, (64, 128), 0) // 32
    c = (jax.lax.broadcasted_iota(jnp.int32, (64, 128), 1) % 64) // 32
    m_kv = r == c
    r2 = jax.lax.broadcasted_iota(jnp.int32, (16, 128), 0) // 8
    c2 = (jax.lax.broadcasted_iota(jnp.int32, (16, 128), 1) % 64) // 32
    m_z = r2 == c2
    ones = jnp.ones((16, 128), BF)
    for pp in range(H // 2):
        kvm = jnp.where(m_kv, kv_ref[pp], 0.0)
        zf = z_ref[pp]
        zh = zf.astype(BF)
        zl = (zf - zh.astype(F32)).astype(BF)
        zt = (jax.lax.dot_general(ones, zh, NT, preferred_element_type=F32)
              + jax.lax.dot_general(ones, zl, NT, preferred_element_type=F32))
        kvl[pp * 40:(pp + 1) * 40, :] = _pk(jnp.concatenate([kvm, jnp.where(m_z, zt, 0.0)], axis=0))

    def body_b(i, carry):
        xcur = xc.at[pl.ds(pl.multiple_of(i * XB, XB), XB), :]
        ow = outv.at[pl.ds(pl.multiple_of(i * L, L), L), :]

        def prod_q(l):
            a = _upk(wq[l * 128:(l + 1) * 128, :])
            b = _upk(xcur[l * (QL // 2):(l + 1) * (QL // 2), :])
            return jax.lax.dot_general(a, b, NT, preferred_element_type=F32)
        blk = _strassen2(prod_q)
        ol = [[] for _ in range(49)]
        for gg in range(8):
            b = gg * 32
            pq = jnp.concatenate([jnp.concatenate([blk[h][c][b:b + 32] for c in range(4)], axis=1)
                                  for h in range(4)], axis=0)
            ep, em = _softmax_pm(pq)
            nd = []
            rc = []
            for p in range(2):
                pp = gg * 2 + p
                phi = jnp.concatenate([ep[p * 64:(p + 1) * 64], em[p * 64:(p + 1) * 64]], axis=0).astype(BF)
                t = jnp.dot(_upk(kvl[pp * 40:(pp + 1) * 40, :]), phi, preferred_element_type=F32)
                rr = pl.reciprocal(t[64:80] + 1e-6, approx=False, full_range=False)
                nd += [t[0:32], t[32:64]]
                rc += [rr[0:8], rr[8:16]]
            for ri in range(2):
                Q = [[None] * 4 for _ in range(4)]
                for h in range(4):
                    o = (nd[h][ri * 16:ri * 16 + 16].reshape(2, 8, L) * rc[h][None]).reshape(16, L)
                    for tq in range(4):
                        Q[tq][h] = o[:, tq * QL:(tq + 1) * QL]

                def emit(l, v):
                    ol[l].append(_pk(v))
                _leaves(Q, _a_combos, emit)
        OA = [None] * 49
        for l in LEAF_ORDER:
            OA[l] = _upk(jnp.concatenate(ol[l], axis=0)).T
        for c in range(OC):
            def prod_o(l, c=c):
                return jnp.dot(OA[l][c * RC:(c + 1) * RC], _upk(wb[l * 128:(l + 1) * 128, :]),
                               preferred_element_type=F32)
            res = _strassen2(prod_o)
            for q in range(4):
                ra = q * QL + c * RC
                for n in range(4):
                    ow[ra:ra + RC, n * 256:(n + 1) * 256] = res[q][n].astype(BF)
                cp_out(i, q, c).start()
        return carry
    jax.lax.fori_loop(0, NB, body_b, 0)
    for i in range(NB):
        for q in range(4):
            for c in range(OC):
                cp_out(i, q, c).wait()


@jax.jit
def pallas_standalone__linear_kernel_hedgehog__prompt_kernel(
    x: jax.Array,
    wqkv: jax.Array,
    w_phi: jax.Array,
    wo: jax.Array,
):
    hbm = pl.BlockSpec(memory_space=pl.ANY)
    out = pl.pallas_call(
        _kernel,
        in_specs=[hbm] * 4,
        out_specs=hbm,
        out_shape=jax.ShapeDtypeStruct((S, D), BF),
        scratch_shapes=[
            pltpu.VMEM((S, D), BF),
            pltpu.VMEM((D, 3 * D), BF),
            pltpu.VMEM((H * DH, DH), BF),
            pltpu.VMEM((D, D), BF),
            pltpu.VMEM((49 * 256, 256), U32),
            pltpu.VMEM((49 * 128, 256), U32),
            pltpu.VMEM((49 * 128, 256), U32),
            pltpu.VMEM(((NB + 1) * XB, 256), U32),
            pltpu.VMEM((8 * 64, 128), U32),
            pltpu.VMEM((H // 2, 64, 128), F32),
            pltpu.VMEM((H // 2, 128, 128), F32),
            pltpu.VMEM((H // 2 * 40, 128), U32),
            pltpu.VMEM((S, D), BF),
            pltpu.SemaphoreType.DMA((NSEM,)),
        ],
        compiler_params=pltpu.CompilerParams(vmem_limit_bytes=110 * 1024 * 1024),
    )(x.reshape(S, D), wqkv, w_phi.reshape(H * DH, DH), wo)
    return out.reshape(1, S, D)
```
